```python
import os as _os
_os.environ.setdefault("JAX_PLATFORMS", "cpu")
import jax
import jax.numpy as jnp

def _softmax(x, axis=-1):
    return jax.nn.softmax(x, axis=axis)
def _gelu(x):
    return jax.nn.gelu(x, approximate=True)
def _silu(x):
    return jax.nn.silu(x)
def _sigmoid(x):
    return jax.nn.sigmoid(x)
def _layernorm(x, axis=-1, eps=1e-5):
    m = jnp.mean(x, axis=axis, keepdims=True)
    v = jnp.var(x, axis=axis, keepdims=True)
    return (x - m) / jnp.sqrt(v + eps)
def _scatter_add(tgt, idx, src, axis=0):
    return tgt.at[idx].add(src)
def _segment_sum(src, seg, n):
    return jax.ops.segment_sum(src, seg, n)
class _Rng:
    def __init__(self, key):
        self._k = key
    def _next(self):
        self._k, sub = jax.random.split(self._k)
        return sub
    def normal(self, shape):
        return jax.random.normal(self._next(), shape, dtype=jnp.bfloat16)
    def randint(self, lo, hi, shape):
        return jax.random.randint(self._next(), shape, lo, hi, dtype=jnp.int32)
    def uniform(self, shape, lo=0.0, hi=1.0):
        return jax.random.uniform(self._next(), shape, jnp.bfloat16, lo, hi)
    def permutation(self, n):
        return jax.random.permutation(self._next(), n)


kernel_name = 'interleave_layers__spectral_gfnet__dense_activation_gelu__prompt'

def setup_inputs():
    _rng = _Rng(jax.random.key(int.from_bytes(__import__("os").urandom(4), "little")))
    _w = (lambda a: (lambda t: t.astype(jnp.bfloat16) if jnp.issubdtype(t.dtype, jnp.floating) else t)(jnp.asarray(a)))
    def _A_setup():
        B, S, D = 1, 2048, 640
        Df = D // 2 + 1
        return {
            "x": _w((lambda *s: _rng.normal(s) * 0.05)(B, S, D)),
            "w_r": _w((lambda *s: _rng.normal(s) * 0.2)(S, Df) * 0.02),
            "w_i": _w((lambda *s: _rng.normal(s) * 0.2)(S, Df) * 0.02),
        }
    _A_in = _A_setup()

    def _B_setup():
        B, S, D, F = 1, 2048, 640, 1728
        return {
            "x": _w((lambda *s: _rng.normal(s) * 0.05)(B, S, D)),
            "w1": _w((lambda *s: _rng.normal(s) * 0.1)(D, F) * (D ** -0.5)),
            "b1": _w((lambda *s: _rng.normal(s) * 0.1)(F) * 0.01),
            "w2": _w((lambda *s: _rng.normal(s) * 0.1)(F, D) * (F ** -0.5)),
            "b2": _w((lambda *s: _rng.normal(s) * 0.1)(D) * 0.01),
        }
    _B_in = _B_setup()

    return {
        "A_x": _A_in["x"],
        "A_w_r": _A_in["w_r"],
        "A_w_i": _A_in["w_i"],
        "B_x": _B_in["x"],
        "B_w1": _B_in["w1"],
        "B_b1": _B_in["b1"],
        "B_w2": _B_in["w2"],
        "B_b2": _B_in["b2"],
    }

def reference(A_x, A_w_r, A_w_i, B_x, B_w1, B_b1, B_w2, B_b2):
    def _A_ref(x, w_r, w_i):
        B, S, D = x.shape
        X = (lambda x, axes=(-2,-1): jnp.fft.rfft2(x.astype(jnp.float32), axes=axes))(x, axes=(-2, -1))
        W = w_r + 1j * w_i
        X = X * W
        y = (lambda x, s, axes=(-2,-1): jnp.fft.irfft2(x, s=s, axes=axes).astype(jnp.bfloat16))(X, (S, D), axes=(-2, -1))
        return y

    def _B_ref(x, w1, b1, w2, b2):
        h = jnp.einsum("bsd,df->bsf", x, w1) + b1
        h = _gelu(h)
        return jnp.einsum("bsf,fd->bsd", h, w2) + b2

    x = A_x
    x = x + _A_ref(_layernorm(x, axis=-1), A_w_r, A_w_i)
    x = x + _B_ref(_layernorm(x, axis=-1), B_w1, B_b1, B_w2, B_b2)
    x = x + _A_ref(_layernorm(x, axis=-1), A_w_r, A_w_i)
    x = x + _B_ref(_layernorm(x, axis=-1), B_w1, B_b1, B_w2, B_b2)
    return x
```

```python
import functools
import math

import numpy as np
import jax
import jax.numpy as jnp
from jax import lax
import jax.experimental.pallas as pl
import jax.experimental.pallas.tpu as pltpu

S = 2048
D = 640
FH = 1728
DF = D // 2 + 1
FP = 384
N1 = 16
N2 = 128
RB = 256
EPS = 1e-5


def _tables():
    d = np.arange(D)[:, None]
    f = np.arange(DF)[None, :]
    ang = 2.0 * np.pi * ((d * f) % D) / D
    fwd = np.zeros((D, 2 * FP), np.float64)
    fwd[:, :DF] = np.cos(ang)
    fwd[:, FP:FP + DF] = -np.sin(ang)
    wgt = np.full((DF,), 2.0)
    wgt[0] = 1.0
    wgt[DF - 1] = 1.0
    inv = np.zeros((2 * FP, D), np.float64)
    inv[:DF, :] = (np.cos(ang) * wgt[None, :]).T
    inv[FP:FP + DF, :] = (-np.sin(ang) * wgt[None, :]).T
    inv /= float(D)
    k1 = np.arange(N1)[:, None, None]
    k2 = np.arange(N2)[None, :, None]
    s2 = np.arange(N2)[None, None, :]
    angs = 2.0 * np.pi * ((s2 * (k1 + N1 * k2)) % S) / S
    c = np.cos(angs)
    sn = np.sin(angs)
    g = np.concatenate([c, sn], axis=1)
    h = np.concatenate([c.transpose(0, 2, 1), sn.transpose(0, 2, 1)], axis=1)
    to_bf = lambda a: jnp.asarray(a.astype(np.float32)).astype(jnp.bfloat16)
    return to_bf(fwd), to_bf(inv), to_bf(g), to_bf(h)


def _cmul_const(a, wr, wi):
    ar, ai = a
    if abs(wr - 1.0) < 1e-12 and abs(wi) < 1e-12:
        return ar, ai
    if abs(wr) < 1e-12 and abs(wi + 1.0) < 1e-12:
        return ai, -ar
    if abs(wr) < 1e-12 and abs(wi - 1.0) < 1e-12:
        return -ai, ar
    return ar * wr - ai * wi, ar * wi + ai * wr


def _fft_list(xs, sign):
    n = len(xs)
    if n == 1:
        return xs
    ev = _fft_list(xs[0::2], sign)
    od = _fft_list(xs[1::2], sign)
    out = [None] * n
    for k in range(n // 2):
        wr = math.cos(2.0 * math.pi * k / n)
        wi = sign * math.sin(2.0 * math.pi * k / n)
        tr, ti = _cmul_const(od[k], wr, wi)
        er, ei = ev[k]
        out[k] = (er + tr, ei + ti)
        out[k + n // 2] = (er - tr, ei - ti)
    return out


def _layernorm_bf16(x):
    m = jnp.mean(x, axis=-1, keepdims=True)
    xc = x - m
    v = jnp.mean(xc * xc, axis=-1, keepdims=True)
    return (xc * lax.rsqrt(v + EPS)).astype(jnp.bfloat16)


def _bf(x):
    return x.astype(jnp.bfloat16).astype(jnp.float32)


def _kernel(x_ref, wr_ref, wi_ref, w1_ref, b1_ref, w2_ref, b2_ref,
            fwd_ref, inv_ref, g_ref, h_ref, o_ref, xs_ref, spec_ref):
    nrb = S // RB

    def d_forward(x):
        xn = _layernorm_bf16(x)
        return jnp.dot(xn, fwd_ref[...], preferred_element_type=jnp.float32)

    def radix16(sign):
        def body(r, carry):
            r0 = pl.multiple_of(r * 8, 8)
            for c in range(FP // 128):
                xs = []
                for j in range(N1):
                    re = spec_ref[pl.ds(j * N2 + r0, 8), pl.ds(c * 128, 128)]
                    im = spec_ref[pl.ds(j * N2 + r0, 8), pl.ds(FP + c * 128, 128)]
                    xs.append((re, im))
                ys = _fft_list(xs, sign)
                for j in range(N1):
                    spec_ref[pl.ds(j * N2 + r0, 8), pl.ds(c * 128, 128)] = ys[j][0]
                    spec_ref[pl.ds(j * N2 + r0, 8), pl.ds(FP + c * 128, 128)] = ys[j][1]
            return carry
        lax.fori_loop(0, N2 // 8, body, 0)

    def spectral_mid():
        def body(k1, carry):
            r0 = pl.multiple_of(k1 * N2, N2)
            t = spec_ref[pl.ds(r0, N2), :].astype(jnp.bfloat16)
            p = jnp.dot(g_ref[k1], t, preferred_element_type=jnp.float32)
            xr = p[:N2, :FP] + p[N2:, FP:]
            xi = p[:N2, FP:] - p[N2:, :FP]
            wr = wr_ref[pl.ds(r0, N2), :].astype(jnp.float32) * (1.0 / S)
            wi = wi_ref[pl.ds(r0, N2), :].astype(jnp.float32) * (1.0 / S)
            yr = xr * wr - xi * wi
            yi = xr * wi + xi * wr
            y = jnp.concatenate([yr, yi], axis=1).astype(jnp.bfloat16)
            q = jnp.dot(h_ref[k1], y, preferred_element_type=jnp.float32)
            spec_ref[pl.ds(r0, N2), pl.ds(0, FP)] = q[:N2, :FP] - q[N2:, FP:]
            spec_ref[pl.ds(r0, N2), pl.ds(FP, FP)] = q[:N2, FP:] + q[N2:, :FP]
            return carry
        lax.fori_loop(0, N1, body, 0)

    def mlp(x):
        xn = _layernorm_bf16(x)
        hh = jnp.dot(xn, w1_ref[...], preferred_element_type=jnp.float32)
        hh = _bf(_bf(hh) + b1_ref[...].astype(jnp.float32))
        hh = jax.nn.gelu(hh, approximate=True).astype(jnp.bfloat16)
        y = jnp.dot(hh, w2_ref[...], preferred_element_type=jnp.float32)
        return _bf(_bf(y) + b2_ref[...].astype(jnp.float32))

    def head(i, carry):
        r0 = pl.multiple_of(i * RB, RB)
        x = x_ref[pl.ds(r0, RB), :].astype(jnp.float32)
        xs_ref[pl.ds(r0, RB), :] = x
        spec_ref[pl.ds(r0, RB), :] = d_forward(x)
        return carry
    lax.fori_loop(0, nrb, head, 0)

    for layer in range(2):
        radix16(-1.0)
        spectral_mid()
        radix16(1.0)

        def tail(i, carry, layer=layer):
            r0 = pl.multiple_of(i * RB, RB)
            z = spec_ref[pl.ds(r0, RB), :].astype(jnp.bfloat16)
            y = jnp.dot(z, inv_ref[...], preferred_element_type=jnp.float32)
            x = _bf(xs_ref[pl.ds(r0, RB), :] + _bf(y))
            x = _bf(x + mlp(x))
            if layer == 0:
                xs_ref[pl.ds(r0, RB), :] = x
                spec_ref[pl.ds(r0, RB), :] = d_forward(x)
            else:
                o_ref[pl.ds(r0, RB), :] = x.astype(o_ref.dtype)
            return carry
        lax.fori_loop(0, nrb, tail, 0)


@jax.jit
def pallas_interleave_layers__spectral_gfnet__dense_activation_gelu__prompt_kernel(
    A_x: jax.Array,
    A_w_r: jax.Array,
    A_w_i: jax.Array,
    B_x: jax.Array,
    B_w1: jax.Array,
    B_b1: jax.Array,
    B_w2: jax.Array,
    B_b2: jax.Array,
):
    x = A_x.reshape(S, D)

    def perm(w):
        w = jnp.pad(w, ((0, 0), (0, FP - DF)))
        return w.reshape(N2, N1, FP).transpose(1, 0, 2).reshape(S, FP)

    wr = perm(A_w_r)
    wi = perm(A_w_i)
    fwd, inv, g, h = _tables()
    out = pl.pallas_call(
        _kernel,
        out_shape=jax.ShapeDtypeStruct((S, D), jnp.bfloat16),
        scratch_shapes=[
            pltpu.VMEM((S, D), jnp.float32),
            pltpu.VMEM((S, 2 * FP), jnp.float32),
        ],
        compiler_params=pltpu.CompilerParams(vmem_limit_bytes=100 * 1024 * 1024),
    )(x, wr, wi, B_w1, B_b1.reshape(1, FH), B_w2, B_b2.reshape(1, D), fwd, inv, g, h)
    return out.reshape(1, S, D)
```

```python
import functools
import math

import numpy as np
import jax
import jax.numpy as jnp
from jax import lax
import jax.experimental.pallas as pl
import jax.experimental.pallas.tpu as pltpu

S = 2048
D = 640
FH = 1728
DF = D // 2 + 1
FP = 384
N1 = 16
N2 = 128
RB = 256
EPS = 1e-5


def _tables():
    d = np.arange(D)[:, None]
    f = np.arange(DF)[None, :]
    ang = 2.0 * np.pi * ((d * f) % D) / D
    fwd = np.zeros((D, 2 * FP), np.float64)
    fwd[:, :DF] = np.cos(ang)
    fwd[:, FP:FP + DF] = -np.sin(ang)
    wgt = np.full((DF,), 2.0)
    wgt[0] = 1.0
    wgt[DF - 1] = 1.0
    inv = np.zeros((2 * FP, D), np.float64)
    inv[:DF, :] = (np.cos(ang) * wgt[None, :]).T
    inv[FP:FP + DF, :] = (-np.sin(ang) * wgt[None, :]).T
    inv /= float(D)
    k1 = np.arange(N1)[:, None, None]
    k2 = np.arange(N2)[None, :, None]
    s2 = np.arange(N2)[None, None, :]
    angs = 2.0 * np.pi * ((s2 * (k1 + N1 * k2)) % S) / S
    c = np.cos(angs)
    sn = np.sin(angs)
    g = np.concatenate([c, sn], axis=1)
    h = np.concatenate([c.transpose(0, 2, 1), sn.transpose(0, 2, 1)], axis=1)
    to_bf = lambda a: jnp.asarray(a.astype(np.float32)).astype(jnp.bfloat16)
    return to_bf(fwd), to_bf(inv), to_bf(g), to_bf(h)


def _cmul_const(a, wr, wi):
    ar, ai = a
    if abs(wr - 1.0) < 1e-12 and abs(wi) < 1e-12:
        return ar, ai
    if abs(wr) < 1e-12 and abs(wi + 1.0) < 1e-12:
        return ai, -ar
    if abs(wr) < 1e-12 and abs(wi - 1.0) < 1e-12:
        return -ai, ar
    return ar * wr - ai * wi, ar * wi + ai * wr


def _fft_list(xs, sign):
    n = len(xs)
    if n == 1:
        return xs
    ev = _fft_list(xs[0::2], sign)
    od = _fft_list(xs[1::2], sign)
    out = [None] * n
    for k in range(n // 2):
        wr = math.cos(2.0 * math.pi * k / n)
        wi = sign * math.sin(2.0 * math.pi * k / n)
        tr, ti = _cmul_const(od[k], wr, wi)
        er, ei = ev[k]
        out[k] = (er + tr, ei + ti)
        out[k + n // 2] = (er - tr, ei - ti)
    return out


def _layernorm_bf16(x):
    m = jnp.mean(x, axis=-1, keepdims=True)
    xc = x - m
    v = jnp.mean(xc * xc, axis=-1, keepdims=True)
    return (xc * lax.rsqrt(v + EPS)).astype(jnp.bfloat16)


def _bf(x):
    return x.astype(jnp.bfloat16).astype(jnp.float32)


def _kernel(x_ref, wr0, wr1, wr2, wi0, wi1, wi2, w1_ref, b1_ref, w2_ref, b2_ref,
            fwd_ref, inv_ref, g_ref, h_ref, o_ref, xs_ref, spec_ref):
    nrb = S // RB

    def d_forward(x):
        xn = _layernorm_bf16(x)
        return jnp.dot(xn, fwd_ref[...], preferred_element_type=jnp.float32)

    def radix16(sign):
        def body(r, carry):
            r0 = pl.multiple_of(r * 8, 8)
            for c in range(FP // 128):
                xs = []
                for j in range(N1):
                    re = spec_ref[pl.ds(j * N2 + r0, 8), pl.ds(c * 128, 128)]
                    im = spec_ref[pl.ds(j * N2 + r0, 8), pl.ds(FP + c * 128, 128)]
                    xs.append((re, im))
                ys = _fft_list(xs, sign)
                for j in range(N1):
                    spec_ref[pl.ds(j * N2 + r0, 8), pl.ds(c * 128, 128)] = ys[j][0]
                    spec_ref[pl.ds(j * N2 + r0, 8), pl.ds(FP + c * 128, 128)] = ys[j][1]
            return carry
        lax.fori_loop(0, N2 // 8, body, 0)

    def spectral_mid():
        def body(k1, carry):
            r0 = pl.multiple_of(k1 * N2, N2)
            t = spec_ref[pl.ds(r0, N2), :].astype(jnp.bfloat16)
            p = jnp.dot(g_ref[k1], t, preferred_element_type=jnp.float32)
            xr = p[:N2, :FP] + p[N2:, FP:]
            xi = p[:N2, FP:] - p[N2:, :FP]
            wr = jnp.concatenate([w[pl.ds(k1, N2, stride=N1), :] for w in (wr0, wr1, wr2)], axis=1) * (1.0 / S)
            wi = jnp.concatenate([w[pl.ds(k1, N2, stride=N1), :] for w in (wi0, wi1, wi2)], axis=1) * (1.0 / S)
            yr = xr * wr - xi * wi
            yi = xr * wi + xi * wr
            y = jnp.concatenate([yr, yi], axis=1).astype(jnp.bfloat16)
            q = jnp.dot(h_ref[k1], y, preferred_element_type=jnp.float32)
            spec_ref[pl.ds(r0, N2), pl.ds(0, FP)] = q[:N2, :FP] - q[N2:, FP:]
            spec_ref[pl.ds(r0, N2), pl.ds(FP, FP)] = q[:N2, FP:] + q[N2:, :FP]
            return carry
        lax.fori_loop(0, N1, body, 0)

    def mlp(x):
        xn = _layernorm_bf16(x)
        hh = jnp.dot(xn, w1_ref[...], preferred_element_type=jnp.float32)
        hh = _bf(_bf(hh) + b1_ref[...].astype(jnp.float32))
        hh = jax.nn.gelu(hh, approximate=True).astype(jnp.bfloat16)
        y = jnp.dot(hh, w2_ref[...], preferred_element_type=jnp.float32)
        return _bf(_bf(y) + b2_ref[...].astype(jnp.float32))

    def head(i, carry):
        r0 = pl.multiple_of(i * RB, RB)
        x = x_ref[pl.ds(r0, RB), :].astype(jnp.float32)
        xs_ref[pl.ds(r0, RB), :] = x
        spec_ref[pl.ds(r0, RB), :] = d_forward(x)
        return carry
    lax.fori_loop(0, nrb, head, 0)

    for layer in range(2):
        radix16(-1.0)
        spectral_mid()
        radix16(1.0)

        def tail(i, carry, layer=layer):
            r0 = pl.multiple_of(i * RB, RB)
            z = spec_ref[pl.ds(r0, RB), :].astype(jnp.bfloat16)
            y = jnp.dot(z, inv_ref[...], preferred_element_type=jnp.float32)
            x = _bf(xs_ref[pl.ds(r0, RB), :] + _bf(y))
            x = _bf(x + mlp(x))
            if layer == 0:
                xs_ref[pl.ds(r0, RB), :] = x
                spec_ref[pl.ds(r0, RB), :] = d_forward(x)
            else:
                o_ref[pl.ds(r0, RB), :] = x.astype(o_ref.dtype)
            return carry
        lax.fori_loop(0, nrb, tail, 0)


@jax.jit
def pallas_interleave_layers__spectral_gfnet__dense_activation_gelu__prompt_kernel(
    A_x: jax.Array,
    A_w_r: jax.Array,
    A_w_i: jax.Array,
    B_x: jax.Array,
    B_w1: jax.Array,
    B_b1: jax.Array,
    B_w2: jax.Array,
    B_b2: jax.Array,
):
    x = A_x.reshape(S, D)

    def perm(w):
        w = jnp.pad(w, ((0, 0), (0, FP - DF))).astype(jnp.float32)
        return [w[:, c * 128:(c + 1) * 128] for c in range(FP // 128)]

    wr = perm(A_w_r)
    wi = perm(A_w_i)
    fwd, inv, g, h = _tables()
    out = pl.pallas_call(
        _kernel,
        out_shape=jax.ShapeDtypeStruct((S, D), jnp.bfloat16),
        scratch_shapes=[
            pltpu.VMEM((S, D), jnp.float32),
            pltpu.VMEM((S, 2 * FP), jnp.float32),
        ],
        compiler_params=pltpu.CompilerParams(vmem_limit_bytes=100 * 1024 * 1024),
    )(x, *wr, *wi, B_w1, B_b1.reshape(1, FH), B_w2, B_b2.reshape(1, D), fwd, inv, g, h)
    return out.reshape(1, S, D)
```

```python
import functools
import math

import numpy as np
import jax
import jax.numpy as jnp
from jax import lax
import jax.experimental.pallas as pl
import jax.experimental.pallas.tpu as pltpu

S = 2048
D = 640
FH = 1728
DF = D // 2 + 1
FP = 384
N1 = 16
N2 = 128
RB = 512
EPS = 1e-5


def _tables():
    d = np.arange(D)[:, None]
    f = np.arange(DF)[None, :]
    ang = 2.0 * np.pi * ((d * f) % D) / D
    fwd = np.zeros((D, 2 * FP), np.float64)
    fwd[:, :DF] = np.cos(ang)
    fwd[:, FP:FP + DF] = -np.sin(ang)
    wgt = np.full((DF,), 2.0)
    wgt[0] = 1.0
    wgt[DF - 1] = 1.0
    inv = np.zeros((2 * FP, D), np.float64)
    inv[:DF, :] = (np.cos(ang) * wgt[None, :]).T
    inv[FP:FP + DF, :] = (-np.sin(ang) * wgt[None, :]).T
    inv /= float(D)
    k1 = np.arange(N1)[:, None, None]
    k2 = np.arange(N2)[None, :, None]
    s2 = np.arange(N2)[None, None, :]
    angs = 2.0 * np.pi * ((s2 * (k1 + N1 * k2)) % S) / S
    c = np.cos(angs)
    sn = np.sin(angs)
    g = np.concatenate([c, sn], axis=1)
    h = np.concatenate([c.transpose(0, 2, 1), sn.transpose(0, 2, 1)], axis=1)
    to_bf = lambda a: jnp.asarray(a.astype(np.float32)).astype(jnp.bfloat16)
    return to_bf(fwd), to_bf(inv), to_bf(g), to_bf(h)


def _cmul_const(a, wr, wi):
    ar, ai = a
    if abs(wr - 1.0) < 1e-12 and abs(wi) < 1e-12:
        return ar, ai
    if abs(wr) < 1e-12 and abs(wi + 1.0) < 1e-12:
        return ai, -ar
    if abs(wr) < 1e-12 and abs(wi - 1.0) < 1e-12:
        return -ai, ar
    return ar * wr - ai * wi, ar * wi + ai * wr


def _fft_list(xs, sign):
    n = len(xs)
    if n == 1:
        return xs
    ev = _fft_list(xs[0::2], sign)
    od = _fft_list(xs[1::2], sign)
    out = [None] * n
    for k in range(n // 2):
        wr = math.cos(2.0 * math.pi * k / n)
        wi = sign * math.sin(2.0 * math.pi * k / n)
        tr, ti = _cmul_const(od[k], wr, wi)
        er, ei = ev[k]
        out[k] = (er + tr, ei + ti)
        out[k + n // 2] = (er - tr, ei - ti)
    return out


def _layernorm_bf16(x):
    m = jnp.mean(x, axis=-1, keepdims=True)
    xc = x - m
    v = jnp.mean(xc * xc, axis=-1, keepdims=True)
    return (xc * lax.rsqrt(v + EPS)).astype(jnp.bfloat16)


def _bf(x):
    return x.astype(jnp.bfloat16).astype(jnp.float32)


def _kernel(x_ref, wr0, wr1, wr2, wi0, wi1, wi2, w1_ref, b1_ref, w2_ref, b2_ref,
            fwd_ref, inv_ref, g_ref, h_ref, o_ref, xs_ref, spec_ref):
    nrb = S // RB

    def d_forward(x):
        xn = _layernorm_bf16(x)
        return jnp.dot(xn, fwd_ref[...], preferred_element_type=jnp.float32)

    def radix16(sign):
        def body(r, carry):
            r0 = pl.multiple_of(r * 8, 8)
            for c in range(FP // 128):
                xs = []
                for j in range(N1):
                    re = spec_ref[pl.ds(j * N2 + r0, 8), pl.ds(c * 128, 128)]
                    im = spec_ref[pl.ds(j * N2 + r0, 8), pl.ds(FP + c * 128, 128)]
                    xs.append((re, im))
                ys = _fft_list(xs, sign)
                for j in range(N1):
                    spec_ref[pl.ds(j * N2 + r0, 8), pl.ds(c * 128, 128)] = ys[j][0]
                    spec_ref[pl.ds(j * N2 + r0, 8), pl.ds(FP + c * 128, 128)] = ys[j][1]
            return carry
        lax.fori_loop(0, N2 // 8, body, 0)

    def spectral_mid():
        def body(k1, carry):
            r0 = pl.multiple_of(k1 * N2, N2)
            t = spec_ref[pl.ds(r0, N2), :].astype(jnp.bfloat16)
            p = jnp.dot(g_ref[k1], t, preferred_element_type=jnp.float32)
            xr = p[:N2, :FP] + p[N2:, FP:]
            xi = p[:N2, FP:] - p[N2:, :FP]
            wr = jnp.concatenate([w[pl.ds(k1, N2, stride=N1), :] for w in (wr0, wr1, wr2)], axis=1) * (1.0 / S)
            wi = jnp.concatenate([w[pl.ds(k1, N2, stride=N1), :] for w in (wi0, wi1, wi2)], axis=1) * (1.0 / S)
            yr = xr * wr - xi * wi
            yi = xr * wi + xi * wr
            y = jnp.concatenate([yr, yi], axis=1).astype(jnp.bfloat16)
            q = jnp.dot(h_ref[k1], y, preferred_element_type=jnp.float32)
            spec_ref[pl.ds(r0, N2), pl.ds(0, FP)] = q[:N2, :FP] - q[N2:, FP:]
            spec_ref[pl.ds(r0, N2), pl.ds(FP, FP)] = q[:N2, FP:] + q[N2:, :FP]
            return carry
        lax.fori_loop(0, N1, body, 0)

    def mlp(x):
        xn = _layernorm_bf16(x)
        hh = lax.dot_general(xn, w1_ref[...], (((1,), (1,)), ((), ())), preferred_element_type=jnp.float32)
        hh = _bf(_bf(hh) + b1_ref[...].astype(jnp.float32))
        hh = jax.nn.gelu(hh, approximate=True).astype(jnp.bfloat16)
        y = jnp.dot(hh, w2_ref[...], preferred_element_type=jnp.float32)
        return _bf(_bf(y) + b2_ref[...].astype(jnp.float32))

    def head(i, carry):
        r0 = pl.multiple_of(i * RB, RB)
        x = x_ref[0, pl.ds(r0, RB), :].astype(jnp.float32)
        xs_ref[pl.ds(r0, RB), :] = x
        spec_ref[pl.ds(r0, RB), :] = d_forward(x)
        return carry
    lax.fori_loop(0, nrb, head, 0)

    for layer in range(2):
        radix16(-1.0)
        spectral_mid()
        radix16(1.0)

        def tail(i, carry, layer=layer):
            r0 = pl.multiple_of(i * RB, RB)
            z = spec_ref[pl.ds(r0, RB), :].astype(jnp.bfloat16)
            y = jnp.dot(z, inv_ref[...], preferred_element_type=jnp.float32)
            x = _bf(xs_ref[pl.ds(r0, RB), :] + _bf(y))
            x = _bf(x + mlp(x))
            if layer == 0:
                xs_ref[pl.ds(r0, RB), :] = x
                spec_ref[pl.ds(r0, RB), :] = d_forward(x)
            else:
                o_ref[0, pl.ds(r0, RB), :] = x.astype(o_ref.dtype)
            return carry
        lax.fori_loop(0, nrb, tail, 0)


@jax.jit
def pallas_interleave_layers__spectral_gfnet__dense_activation_gelu__prompt_kernel(
    A_x: jax.Array,
    A_w_r: jax.Array,
    A_w_i: jax.Array,
    B_x: jax.Array,
    B_w1: jax.Array,
    B_b1: jax.Array,
    B_w2: jax.Array,
    B_b2: jax.Array,
):
    x = A_x

    def perm(w):
        w = jnp.pad(w, ((0, 0), (0, FP - DF))).astype(jnp.float32)
        return [w[:, c * 128:(c + 1) * 128] for c in range(FP // 128)]

    wr = perm(A_w_r)
    wi = perm(A_w_i)
    fwd, inv, g, h = _tables()
    out = pl.pallas_call(
        _kernel,
        out_shape=jax.ShapeDtypeStruct((1, S, D), jnp.bfloat16),
        scratch_shapes=[
            pltpu.VMEM((S, D), jnp.float32),
            pltpu.VMEM((S, 2 * FP), jnp.float32),
        ],
        compiler_params=pltpu.CompilerParams(vmem_limit_bytes=100 * 1024 * 1024),
    )(x, *wr, *wi, B_w1.T, B_b1.reshape(1, FH), B_w2, B_b2.reshape(1, D), fwd, inv, g, h)
    return out
```
